```python
import os as _os
_os.environ.setdefault("JAX_PLATFORMS", "cpu")
import jax
import jax.numpy as jnp

def _softmax(x, axis=-1):
    return jax.nn.softmax(x, axis=axis)
def _gelu(x):
    return jax.nn.gelu(x, approximate=True)
def _silu(x):
    return jax.nn.silu(x)
def _sigmoid(x):
    return jax.nn.sigmoid(x)
def _layernorm(x, axis=-1, eps=1e-5):
    m = jnp.mean(x, axis=axis, keepdims=True)
    v = jnp.var(x, axis=axis, keepdims=True)
    return (x - m) / jnp.sqrt(v + eps)
def _scatter_add(tgt, idx, src, axis=0):
    return tgt.at[idx].add(src)
def _segment_sum(src, seg, n):
    return jax.ops.segment_sum(src, seg, n)
class _Rng:
    def __init__(self, key):
        self._k = key
    def _next(self):
        self._k, sub = jax.random.split(self._k)
        return sub
    def normal(self, shape):
        return jax.random.normal(self._next(), shape, dtype=jnp.bfloat16)
    def randint(self, lo, hi, shape):
        return jax.random.randint(self._next(), shape, lo, hi, dtype=jnp.int32)
    def uniform(self, shape, lo=0.0, hi=1.0):
        return jax.random.uniform(self._next(), shape, jnp.bfloat16, lo, hi)
    def permutation(self, n):
        return jax.random.permutation(self._next(), n)


kernel_name = 'standalone__mha_softmax__sampling'

def setup_inputs():
    _rng = _Rng(jax.random.key(int.from_bytes(__import__("os").urandom(4), "little")))
    _w = (lambda a: (lambda t: t.astype(jnp.bfloat16) if jnp.issubdtype(t.dtype, jnp.floating) else t)(jnp.asarray(a)))
    B, H, Sq, Sk, D = 8, 32, 32, 2048, 128
    return {
        "q": _w((lambda *s: _rng.normal(s) * 0.4)(B, H, Sq, D)),
        "k": _w((lambda *s: _rng.normal(s) * 0.4)(B, H, Sk, D)),
        "v": _w((lambda *s: _rng.normal(s) * 0.05)(B, H, Sk, D)),
    }

def reference(q, k, v):
    scale = q.shape[-1] ** -0.5
    scores = jnp.einsum("bhqd,bhkd->bhqk", q, k) * scale
    p = _softmax(scores, axis=-1)
    return jnp.einsum("bhqk,bhkd->bhqd", p, v)
```

```python
import functools

import jax
import jax.numpy as jnp
import jax.experimental.pallas as pl
import jax.experimental.pallas.tpu as pltpu


def _kernel(q_ref, k_ref, v_ref, o_ref, *, hb, scale):
    for h in range(hb):
        q = q_ref[h]
        k = k_ref[h]
        v = v_ref[h]
        s = jax.lax.dot_general(q, k, (((1,), (1,)), ((), ())),
                                preferred_element_type=jnp.float32)
        m = jnp.max(s, axis=-1, keepdims=True)
        p = jnp.exp((s - m) * scale)
        l = jnp.sum(p, axis=-1, keepdims=True)
        o = jnp.dot(p.astype(jnp.bfloat16), v, preferred_element_type=jnp.float32)
        o_ref[h] = (o / l).astype(o_ref.dtype)


@jax.jit
def pallas_standalone__mha_softmax__sampling_kernel(
    q: jax.Array,
    k: jax.Array,
    v: jax.Array,
):
    B, H, Sq, D = q.shape
    Sk = k.shape[2]
    BH = B * H
    hb = 4
    q3 = q.reshape(BH, Sq, D)
    k3 = k.reshape(BH, Sk, D)
    v3 = v.reshape(BH, Sk, D)
    out = pl.pallas_call(
        functools.partial(_kernel, hb=hb, scale=D ** -0.5),
        grid=(BH // hb,),
        in_specs=[
            pl.BlockSpec((hb, Sq, D), lambda i: (i, 0, 0)),
            pl.BlockSpec((hb, Sk, D), lambda i: (i, 0, 0)),
            pl.BlockSpec((hb, Sk, D), lambda i: (i, 0, 0)),
        ],
        out_specs=pl.BlockSpec((hb, Sq, D), lambda i: (i, 0, 0)),
        out_shape=jax.ShapeDtypeStruct((BH, Sq, D), q.dtype),
        compiler_params=pltpu.CompilerParams(
            dimension_semantics=("arbitrary",),
            vmem_limit_bytes=64 * 1024 * 1024,
        ),
    )(q3, k3, v3)
    return out.reshape(B, H, Sq, D)
```

```python
import functools

import jax
import jax.numpy as jnp
import jax.experimental.pallas as pl
import jax.experimental.pallas.tpu as pltpu

_G = 2
_DEPTH = 4
_BLK = 256
_HEAD = 16


def _kernel(q_hbm, k_hbm, v_hbm, o_hbm, qbuf, kbuf, vbuf, obuf,
            qsem, ksem, vsem, osem, *, ngroups, sk, scale):
    G, depth = _G, _DEPTH

    def head(g, h):
        return g + h * ngroups

    def issue_group(g, slot):
        for h in range(G):
            pltpu.make_async_copy(
                q_hbm.at[head(g, h)], qbuf.at[slot, h], qsem.at[slot]
            ).start(priority=0)
        for j in range(sk // _BLK):
            for h in range(G):
                for src, dst, sem in ((k_hbm, kbuf, ksem), (v_hbm, vbuf, vsem)):
                    for prio, (o, n) in enumerate(
                        ((j * _BLK, _HEAD), (j * _BLK + _HEAD, _BLK - _HEAD))
                    ):
                        pltpu.make_async_copy(
                            src.at[head(g, h), pl.ds(o, n)],
                            dst.at[slot, h, pl.ds(o, n)],
                            sem.at[slot],
                        ).start(priority=prio)

    def wait_group(slot):
        for buf, sem in ((qbuf, qsem), (kbuf, ksem), (vbuf, vsem)):
            pltpu.make_async_copy(buf.at[slot], buf.at[slot], sem.at[slot]).wait()

    def write_groups(g0, n):
        for h in range(G):
            rows = pl.ds(head(g0, h), n)
            pltpu.make_async_copy(obuf.at[rows], o_hbm.at[rows], osem.at[0]).start()

    def compute(g, slot):
        for h in range(G):
            q = qbuf[slot, h]
            k = kbuf[slot, h]
            v = vbuf[slot, h]
            s = jax.lax.dot_general(q, k, (((1,), (1,)), ((), ())),
                                    preferred_element_type=jnp.float32)
            m = jnp.max(s, axis=-1, keepdims=True)
            p = jnp.exp((s - m) * scale)
            l = jnp.sum(p, axis=-1, keepdims=True)
            o = jnp.dot(p.astype(jnp.bfloat16), v,
                        preferred_element_type=jnp.float32)
            obuf[head(g, h)] = (o / l).astype(obuf.dtype)

    def body(t, carry):
        @pl.when(t < ngroups)
        def _():
            issue_group(t, t % depth)

        i = t - (depth - 1)

        @pl.when(i >= 0)
        def _():
            slot = i % depth
            wait_group(slot)

            @pl.when(i == ngroups - 1)
            def _():
                write_groups(0, ngroups - 1)

            compute(i, slot)

        return carry

    jax.lax.fori_loop(0, ngroups + depth - 1, body, 0)
    write_groups(ngroups - 1, 1)
    pltpu.make_async_copy(obuf, obuf, osem.at[0]).wait()


@jax.jit
def pallas_standalone__mha_softmax__sampling_kernel(
    q: jax.Array,
    k: jax.Array,
    v: jax.Array,
):
    B, H, Sq, D = q.shape
    Sk = k.shape[2]
    BH = B * H
    q3 = q.reshape(BH, Sq, D)
    k3 = k.reshape(BH, Sk, D)
    v3 = v.reshape(BH, Sk, D)
    out = pl.pallas_call(
        functools.partial(_kernel, ngroups=BH // _G, sk=Sk, scale=D ** -0.5),
        in_specs=[pl.BlockSpec(memory_space=pl.ANY)] * 3,
        out_specs=pl.BlockSpec(memory_space=pl.ANY),
        out_shape=jax.ShapeDtypeStruct((BH, Sq, D), q.dtype),
        scratch_shapes=[
            pltpu.VMEM((_DEPTH, _G, Sq, D), q.dtype),
            pltpu.VMEM((_DEPTH, _G, Sk, D), k.dtype),
            pltpu.VMEM((_DEPTH, _G, Sk, D), v.dtype),
            pltpu.VMEM((BH, Sq, D), q.dtype),
            pltpu.SemaphoreType.DMA((_DEPTH,)),
            pltpu.SemaphoreType.DMA((_DEPTH,)),
            pltpu.SemaphoreType.DMA((_DEPTH,)),
            pltpu.SemaphoreType.DMA((1,)),
        ],
        compiler_params=pltpu.CompilerParams(
            vmem_limit_bytes=64 * 1024 * 1024,
            disable_bounds_checks=True,
        ),
    )(q3, k3, v3)
    return out.reshape(B, H, Sq, D)
```

```python
import functools

import jax
import jax.numpy as jnp
from jax import lax
import jax.experimental.pallas as pl
import jax.experimental.pallas.tpu as pltpu

_BLK = 256
_LEAD = 16
_PHASE = 96
_NL = 8
_SLOTS = 16
_LOOK = 3
_MUL = 3
_PENDING = 4
_TRIG = 2


def _kernel(q_hbm, k_hbm, v_hbm, o_hbm, qbuf, kvbuf, obuf, sem, qosem, *,
            nh, sq, sk, scale):
    per = nh // _NL
    lane_rows = per * sq
    nw = nh - _PENDING
    trig = nw + _TRIG - 1

    def lane(n):
        return (n * _MUL) & (_NL - 1)

    def head(n):
        return lane(n) * per + (n >> 3)

    def kv_copy(which, n, off, rows, prio):
        src = (k_hbm, v_hbm)[which]
        slot = n & (_SLOTS - 1)
        pltpu.make_async_copy(
            src.at[head(n), pl.ds(off, rows)],
            kvbuf.at[slot, which, pl.ds(off, rows)],
            sem.at[slot],
        ).start(priority=prio)

    def issue_round(r, carry):
        def full_block(j, c):
            off = pl.multiple_of(_PHASE + _BLK * (j - 1), 32)
            off2 = pl.multiple_of(off + _LEAD, 16)
            for which in range(2):
                kv_copy(which, r - j, off, _LEAD, 0)
                kv_copy(which, r - j, off2, _BLK - _LEAD, 1)
            return c

        lax.fori_loop(jnp.maximum(1, r - (nh - 1)), jnp.minimum(_NL, r + 1),
                      full_block, 0)
        off = _PHASE + _BLK * (_NL - 1)
        for which in range(2):
            @pl.when(r >= _NL)
            def _():
                kv_copy(which, r - _NL, off, _LEAD, 0)
                kv_copy(which, r - _NL, off + _LEAD, sk - off - _LEAD, 1)

            @pl.when(r < nh)
            def _():
                kv_copy(which, r, 0, _PHASE, 1)
        return carry

    def q_copy(off, rows, prio):
        pltpu.make_async_copy(
            q_hbm.at[pl.ds(off, rows)], qbuf.at[pl.ds(off, rows)], qosem.at[0]
        ).start(priority=prio)

    nqb = nh * sq // _BLK

    def q_block(i, c):
        idx = (i & 3) * (nqb // 4) + (i >> 2)
        off = pl.multiple_of(_PHASE + idx * _BLK, 32)
        q_copy(off, _LEAD, 0)
        q_copy(pl.multiple_of(off + _LEAD, 16), _BLK - _LEAD, 1)
        return c

    def wait_kv(n, c):
        slot = n & (_SLOTS - 1)
        pltpu.make_async_copy(kvbuf.at[slot], kvbuf.at[slot], sem.at[slot]).wait()
        return c

    def o_copy(idx):
        pltpu.make_async_copy(obuf.at[idx], o_hbm.at[idx], qosem.at[0]).start()

    def write_piece(i, c):
        rows = pl.ds(pl.multiple_of((i >> 1) * _BLK, _BLK), _BLK)
        o_copy((slice(None), i & 1, rows))
        return c

    def write_last(n):
        l = lane(n)
        o_copy((l >> 1, l & 1, pl.ds(lane_rows - sq, sq)))

    def compute(n):
        l = lane(n)
        slot = n & (_SLOTS - 1)
        q = qbuf[pl.ds(pl.multiple_of(head(n) * sq, sq), sq), :]
        k = kvbuf[slot, 0]
        v = kvbuf[slot, 1]
        s = lax.dot_general(q, k, (((1,), (1,)), ((), ())),
                            preferred_element_type=jnp.float32)
        m = jnp.max(s, axis=-1, keepdims=True)
        p = jnp.exp((s - m) * scale)
        denom = jnp.sum(p, axis=-1, keepdims=True)
        o = jnp.dot(p.astype(jnp.bfloat16), v, preferred_element_type=jnp.float32)
        rows = pl.ds(pl.multiple_of((n >> 3) * sq, sq), sq)
        obuf[l >> 1, l & 1, rows, :] = (o / denom).astype(obuf.dtype)

    lag = _NL + _LOOK
    nrounds = nh + _NL
    nfull = lane_rows // _BLK - 1

    q_copy(0, _PHASE, 1)
    lax.fori_loop(0, nqb - 1, q_block, 0)
    q_copy(_PHASE + (nqb - 1) * _BLK, _BLK - _PHASE, 1)
    lax.fori_loop(0, lag, issue_round, 0)
    pltpu.make_async_copy(qbuf, qbuf, qosem.at[0]).wait()

    def body(n, carry):
        t = n + lag
        lax.fori_loop(t, jnp.minimum(t + 1, nrounds), issue_round, 0)
        whi = jnp.where(
            n == nw, trig + 1,
            jnp.where(jnp.logical_and(n > nw, n <= trig), n, n + 1))
        lax.fori_loop(n, whi, wait_kv, 0)
        lax.fori_loop(0, jnp.where(n == nw, 2 * nfull, 0), write_piece, 0)

        @pl.when(n == nw)
        def _():
            for h in range(2):
                o_copy((slice(None), h, pl.ds(nfull * _BLK, _BLK - sq)))
            for m in range(nh - _NL, nw):
                write_last(m)

        compute(n)

        @pl.when(n >= nw)
        def _():
            write_last(n)

        return carry

    lax.fori_loop(0, nh, body, 0)
    pltpu.make_async_copy(obuf, obuf, qosem.at[0]).wait()


def _params():
    kw = dict(vmem_limit_bytes=48 * 1024 * 1024, disable_bounds_checks=True)
    try:
        return pltpu.CompilerParams(disable_semaphore_checks=True, **kw)
    except TypeError:
        return pltpu.CompilerParams(**kw)


@jax.jit
def pallas_standalone__mha_softmax__sampling_kernel(
    q: jax.Array,
    k: jax.Array,
    v: jax.Array,
):
    B, H, Sq, D = q.shape
    Sk = k.shape[2]
    nh = B * H
    assert Sk == _NL * _BLK and nh % _NL == 0 and (nh // _NL * Sq) % _BLK == 0
    oshape = (_NL // 2, 2, nh // _NL * Sq, D)
    out = pl.pallas_call(
        functools.partial(_kernel, nh=nh, sq=Sq, sk=Sk, scale=D ** -0.5),
        in_specs=[pl.BlockSpec(memory_space=pl.ANY)] * 3,
        out_specs=pl.BlockSpec(memory_space=pl.ANY),
        out_shape=jax.ShapeDtypeStruct(oshape, q.dtype),
        scratch_shapes=[
            pltpu.VMEM((nh * Sq, D), q.dtype),
            pltpu.VMEM((_SLOTS, 2, Sk, D), k.dtype),
            pltpu.VMEM(oshape, q.dtype),
            pltpu.SemaphoreType.DMA((_SLOTS,)),
            pltpu.SemaphoreType.DMA((1,)),
        ],
        compiler_params=_params(),
    )(q.reshape(nh * Sq, D), k.reshape(nh, Sk, D), v.reshape(nh, Sk, D))
    return out.reshape(B, H, Sq, D)
```

```python
import functools

import jax
import jax.numpy as jnp
from jax import lax
import jax.experimental.pallas as pl
import jax.experimental.pallas.tpu as pltpu

_BLK = 256
_LEAD = (24, 16)
_PHASE = 104
_NL = 8
_SLOTS = 16
_LOOK = 3
_VLAG = 2
_MUL = 5
_QPER = 4
_PENDING = 4


def _kernel(q_hbm, k_hbm, v_hbm, o_hbm, qbuf, kvbuf, obuf, sem, qosem, *,
            nh, sq, sk, scale):
    per = nh // _NL
    lane_rows = per * sq
    nw = nh - _PENDING

    def lane(n):
        return (n * _MUL) & (_NL - 1)

    def head(n):
        return lane(n) * per + (n >> 3)

    def kv_copy(which, n, off, rows, prio):
        src = (k_hbm, v_hbm)[which]
        slot = n & (_SLOTS - 1)
        pltpu.make_async_copy(
            src.at[head(n), pl.ds(off, rows)],
            kvbuf.at[slot, which, pl.ds(off, rows)],
            sem.at[slot],
        ).start(priority=prio)

    def full_blocks(t, arrays, descending):
        def body(i, c):
            j = _NL - i if descending else i
            off = pl.multiple_of(_PHASE + _BLK * (j - 1), 8)
            for which in arrays:
                n = t - which * _VLAG - j
                lead = _LEAD[which]
                kv_copy(which, n, off, lead, 0)
                kv_copy(which, n, pl.multiple_of(off + lead, 8), _BLK - lead, 1)
            return c
        return body

    def end_blocks(t, which):
        r = t - which * _VLAG
        off = _PHASE + _BLK * (_NL - 1)
        lead = _LEAD[which]

        @pl.when(jnp.logical_and(r >= _NL, r < nh + _NL))
        def _():
            kv_copy(which, r - _NL, off, lead, 0)
            kv_copy(which, r - _NL, off + lead, sk - off - lead, 1)

        @pl.when(jnp.logical_and(r >= 0, r < nh))
        def _():
            kv_copy(which, r, 0, _PHASE, 1)

    def issue_step(t, carry):
        vhi = jnp.clip(t - _VLAG + 1, 1, _NL)
        lax.fori_loop(1, vhi, full_blocks(t, (0, 1), False), 0)
        lax.fori_loop(vhi, jnp.minimum(_NL, t + 1), full_blocks(t, (0,), False), 0)
        end_blocks(t, 0)
        end_blocks(t, 1)
        return carry

    def issue_drain_step(t, carry):
        end_blocks(t, 1)
        end_blocks(t, 0)
        khi = _NL + 1 - jnp.minimum(t - (nh - 1), _NL)
        vhi = _NL + 1 - jnp.maximum(t - _VLAG - (nh - 1), 1)
        lax.fori_loop(1, khi, full_blocks(t, (1, 0), True), 0)
        lax.fori_loop(khi, vhi, full_blocks(t, (1,), True), 0)
        return carry

    def q_copy(off, rows, prio):
        pltpu.make_async_copy(
            q_hbm.at[pl.ds(off, rows)], qbuf.at[pl.ds(off, rows)], qosem.at[0]
        ).start(priority=prio)

    nqb = nh * sq // _BLK

    def q_block(i, c):
        idx = (i & 3) * (nqb // 4) + (i >> 2)
        off = pl.multiple_of(_PHASE + idx * _BLK, 8)
        q_copy(off, _LEAD[0], 0)
        q_copy(pl.multiple_of(off + _LEAD[0], 8), _BLK - _LEAD[0], 1)
        return c

    def ramp_step(t, carry):
        lax.fori_loop(jnp.minimum(t * _QPER, nqb - 1),
                      jnp.minimum((t + 1) * _QPER, nqb - 1), q_block, 0)
        return issue_step(t, carry)

    def o_copy(idx):
        pltpu.make_async_copy(obuf.at[idx], o_hbm.at[idx], qosem.at[0]).start()

    def write_piece(i, c):
        rows = pl.ds(pl.multiple_of((i >> 1) * _BLK, _BLK), _BLK)
        o_copy((slice(None), i & 1, rows))
        return c

    def write_last(n):
        l = lane(n)
        o_copy((l >> 1, l & 1, pl.ds(lane_rows - sq, sq)))

    def compute(n):
        l = lane(n)
        slot = n & (_SLOTS - 1)
        q = qbuf[pl.ds(pl.multiple_of(head(n) * sq, sq), sq), :]
        k = kvbuf[slot, 0]
        v = kvbuf[slot, 1]
        s = lax.dot_general(q, k, (((1,), (1,)), ((), ())),
                            preferred_element_type=jnp.float32)
        m = jnp.max(s, axis=-1, keepdims=True)
        p = jnp.exp((s - m) * scale)
        denom = jnp.sum(p, axis=-1, keepdims=True)
        o = jnp.dot(p.astype(jnp.bfloat16), v, preferred_element_type=jnp.float32)
        rows = pl.ds(pl.multiple_of((n >> 3) * sq, sq), sq)
        obuf[l >> 1, l & 1, rows, :] = (o / denom).astype(obuf.dtype)

    lag = _NL + _VLAG + _LOOK
    nsteps = nh + _NL + _VLAG
    nfull = lane_rows // _BLK - 1
    assert lag < _SLOTS and lag * _QPER >= nqb - 1

    q_copy(0, _PHASE, 1)
    q_copy(_PHASE + (nqb - 1) * _BLK, _BLK - _PHASE, 1)
    lax.fori_loop(0, lag, ramp_step, 0)
    pltpu.make_async_copy(qbuf, qbuf, qosem.at[0]).wait()

    def body(n, carry):
        t = n + lag
        lax.fori_loop(t, jnp.minimum(t + 1, nh), issue_step, 0)
        lax.fori_loop(jnp.maximum(t, nh), jnp.minimum(t + 1, nsteps),
                      issue_drain_step, 0)
        slot = n & (_SLOTS - 1)
        pltpu.make_async_copy(kvbuf.at[slot], kvbuf.at[slot], sem.at[slot]).wait()
        lax.fori_loop(0, jnp.where(n == nw, 2 * nfull, 0), write_piece, 0)

        @pl.when(n == nw)
        def _():
            for h in range(2):
                o_copy((slice(None), h, pl.ds(nfull * _BLK, _BLK - sq)))
            for m in range(nh - _NL, nw):
                write_last(m)

        compute(n)

        @pl.when(n >= nw)
        def _():
            write_last(n)

        return carry

    lax.fori_loop(0, nh, body, 0)
    pltpu.make_async_copy(obuf, obuf, qosem.at[0]).wait()


def _params():
    kw = dict(vmem_limit_bytes=48 * 1024 * 1024, disable_bounds_checks=True)
    try:
        return pltpu.CompilerParams(disable_semaphore_checks=True, **kw)
    except TypeError:
        return pltpu.CompilerParams(**kw)


@jax.jit
def pallas_standalone__mha_softmax__sampling_kernel(
    q: jax.Array,
    k: jax.Array,
    v: jax.Array,
):
    B, H, Sq, D = q.shape
    Sk = k.shape[2]
    nh = B * H
    assert Sk == _NL * _BLK and nh % _NL == 0 and (nh // _NL * Sq) % _BLK == 0
    oshape = (_NL // 2, 2, nh // _NL * Sq, D)
    out = pl.pallas_call(
        functools.partial(_kernel, nh=nh, sq=Sq, sk=Sk, scale=D ** -0.5),
        in_specs=[pl.BlockSpec(memory_space=pl.ANY)] * 3,
        out_specs=pl.BlockSpec(memory_space=pl.ANY),
        out_shape=jax.ShapeDtypeStruct(oshape, q.dtype),
        scratch_shapes=[
            pltpu.VMEM((nh * Sq, D), q.dtype),
            pltpu.VMEM((_SLOTS, 2, Sk, D), k.dtype),
            pltpu.VMEM(oshape, q.dtype),
            pltpu.SemaphoreType.DMA((_SLOTS,)),
            pltpu.SemaphoreType.DMA((1,)),
        ],
        compiler_params=_params(),
    )(q.reshape(nh * Sq, D), k.reshape(nh, Sk, D), v.reshape(nh, Sk, D))
    return out.reshape(B, H, Sq, D)
```

```python
import functools

import jax
import jax.numpy as jnp
from jax import lax
import jax.experimental.pallas as pl
import jax.experimental.pallas.tpu as pltpu

_BLK = 256
_LEAD = 24
_DELAY = 12
_PHASE = 104
_NL = 8
_SLOTS = 16
_LOOK = 3
_VLAG = 2
_MUL = 5
_QPER = 4
_PENDING = 4


def _kernel(q_hbm, k_hbm, v_hbm, o_hbm, qbuf, kvbuf, obuf, sem, qosem, *,
            nh, sq, sk, scale):
    per = nh // _NL
    lane_rows = per * sq
    nw = nh - _PENDING

    def lane(n):
        return (n * _MUL) & (_NL - 1)

    def head(n):
        return lane(n) * per + (n >> 3)

    def kv_copy(which, n, off, rows, prio):
        src = (k_hbm, v_hbm)[which]
        slot = n & (_SLOTS - 1)
        pltpu.make_async_copy(
            src.at[head(n), pl.ds(off, rows)],
            kvbuf.at[slot, which, pl.ds(off, rows)],
            sem.at[slot],
        ).start(priority=prio)

    tail = _PHASE + _BLK * (_NL - 1)

    def when_started(n, ramp):
        return pl.when(n >= 0) if ramp else (lambda f: f())

    def lead_at(pos, which, ramp):
        jm1 = pos & (_NL - 1)
        n = (pos >> 3) - which * _VLAG - jm1 - 1

        @when_started(n, ramp)
        def _():
            kv_copy(which, n, pl.multiple_of(_PHASE + _BLK * jm1, 8), _LEAD, 0)

    def issue_step(t, ramp):
        def full_block(j, c):
            off = pl.multiple_of(_PHASE + _LEAD + _BLK * (j - 1), 8)
            for which in range(2):
                lead_at(_NL * t + j - 1 - _DELAY, which, ramp)
                n = t - which * _VLAG - j

                @when_started(n, ramp)
                def _():
                    kv_copy(which, n, off, _BLK - _LEAD, 1)
            return c

        lax.fori_loop(1, _NL, full_block, 0)
        for which in range(2):
            r = t - which * _VLAG
            lead_at(_NL * t + _NL - 1 - _DELAY, which, ramp)

            @when_started(r - _NL, ramp)
            def _():
                kv_copy(which, r - _NL, tail + _LEAD, sk - tail - _LEAD, 1)

            @when_started(r, ramp)
            def _():
                kv_copy(which, r, 0, _PHASE, 1)

    def steady_step(t, carry):
        issue_step(t, False)
        return carry

    def flush_leads(pos, carry):
        for which in range(2):
            lead_at(pos, which, False)
        return carry

    def drain_blocks(t, arrays):
        def body(i, c):
            j = _NL - i
            off = pl.multiple_of(_PHASE + _BLK * (j - 1), 8)
            for which in arrays:
                n = t - which * _VLAG - j
                kv_copy(which, n, off, _LEAD, 0)
                kv_copy(which, n, pl.multiple_of(off + _LEAD, 8), _BLK - _LEAD, 1)
            return c
        return body

    def drain_step(t, carry):
        kv_copy(1, t - _VLAG - _NL, tail, _LEAD, 0)
        kv_copy(1, t - _VLAG - _NL, tail + _LEAD, sk - tail - _LEAD, 1)

        @pl.when(t - _VLAG < nh)
        def _():
            kv_copy(1, t - _VLAG, 0, _PHASE, 1)

        @pl.when(t < nh + _NL)
        def _():
            kv_copy(0, t - _NL, tail, _LEAD, 0)
            kv_copy(0, t - _NL, tail + _LEAD, sk - tail - _LEAD, 1)

        khi = _NL + 1 - jnp.minimum(t - (nh - 1), _NL)
        vhi = _NL + 1 - jnp.maximum(t - _VLAG - (nh - 1), 1)
        lax.fori_loop(1, khi, drain_blocks(t, (1, 0)), 0)
        lax.fori_loop(khi, vhi, drain_blocks(t, (1,)), 0)
        return carry

    def q_copy(off, rows, prio):
        pltpu.make_async_copy(
            q_hbm.at[pl.ds(off, rows)], qbuf.at[pl.ds(off, rows)], qosem.at[0]
        ).start(priority=prio)

    nqb = nh * sq // _BLK

    def q_block(i, c):
        idx = (i & 3) * (nqb // 4) + (i >> 2)
        off = pl.multiple_of(_PHASE + idx * _BLK, 8)
        q_copy(off, _LEAD, 0)
        q_copy(pl.multiple_of(off + _LEAD, 8), _BLK - _LEAD, 1)
        return c

    def ramp_step(t, carry):
        lax.fori_loop(jnp.minimum(t * _QPER, nqb - 1),
                      jnp.minimum((t + 1) * _QPER, nqb - 1), q_block, 0)
        issue_step(t, True)
        return carry

    def o_copy(idx):
        pltpu.make_async_copy(obuf.at[idx], o_hbm.at[idx], qosem.at[0]).start()

    def write_piece(i, c):
        rows = pl.ds(pl.multiple_of((i >> 1) * _BLK, _BLK), _BLK)
        o_copy((slice(None), i & 1, rows))
        return c

    def write_last(n):
        l = lane(n)
        o_copy((l >> 1, l & 1, pl.ds(lane_rows - sq, sq)))

    def compute(n):
        l = lane(n)
        slot = n & (_SLOTS - 1)
        q = qbuf[pl.ds(pl.multiple_of(head(n) * sq, sq), sq), :]
        k = kvbuf[slot, 0]
        v = kvbuf[slot, 1]
        s = lax.dot_general(q, k, (((1,), (1,)), ((), ())),
                            preferred_element_type=jnp.float32)
        m = jnp.max(s, axis=-1, keepdims=True)
        p = jnp.exp((s - m) * scale)
        denom = jnp.sum(p, axis=-1, keepdims=True)
        o = jnp.dot(p.astype(jnp.bfloat16), v, preferred_element_type=jnp.float32)
        rows = pl.ds(pl.multiple_of((n >> 3) * sq, sq), sq)
        obuf[l >> 1, l & 1, rows, :] = (o / denom).astype(obuf.dtype)

    lag = _NL + _VLAG + _LOOK
    nsteps = nh + _NL + _VLAG
    nfull = lane_rows // _BLK - 1
    assert lag < _SLOTS and lag * _QPER >= nqb - 1 and _DELAY <= _NL * _LOOK

    q_copy(0, _PHASE, 1)
    q_copy(_PHASE + (nqb - 1) * _BLK, _BLK - _PHASE, 1)
    lax.fori_loop(0, lag, ramp_step, 0)
    pltpu.make_async_copy(qbuf, qbuf, qosem.at[0]).wait()

    def body(n, carry):
        t = n + lag
        lax.fori_loop(t, jnp.minimum(t + 1, nh), steady_step, 0)
        lax.fori_loop(_NL * nh - _DELAY, jnp.where(t == nh - 1, _NL * nh, 0),
                      flush_leads, 0)
        lax.fori_loop(jnp.maximum(t, nh), jnp.minimum(t + 1, nsteps), drain_step, 0)
        slot = n & (_SLOTS - 1)
        pltpu.make_async_copy(kvbuf.at[slot], kvbuf.at[slot], sem.at[slot]).wait()
        lax.fori_loop(0, jnp.where(n == nw, 2 * nfull, 0), write_piece, 0)

        @pl.when(n == nw)
        def _():
            for h in range(2):
                o_copy((slice(None), h, pl.ds(nfull * _BLK, _BLK - sq)))
            for m in range(nh - _NL, nw):
                write_last(m)

        compute(n)

        @pl.when(n >= nw)
        def _():
            write_last(n)

        return carry

    lax.fori_loop(0, nh, body, 0)
    pltpu.make_async_copy(obuf, obuf, qosem.at[0]).wait()


def _params():
    kw = dict(vmem_limit_bytes=48 * 1024 * 1024, disable_bounds_checks=True)
    try:
        return pltpu.CompilerParams(disable_semaphore_checks=True, **kw)
    except TypeError:
        return pltpu.CompilerParams(**kw)


@jax.jit
def pallas_standalone__mha_softmax__sampling_kernel(
    q: jax.Array,
    k: jax.Array,
    v: jax.Array,
):
    B, H, Sq, D = q.shape
    Sk = k.shape[2]
    nh = B * H
    assert Sk == _NL * _BLK and nh % _NL == 0 and (nh // _NL * Sq) % _BLK == 0
    oshape = (_NL // 2, 2, nh // _NL * Sq, D)
    out = pl.pallas_call(
        functools.partial(_kernel, nh=nh, sq=Sq, sk=Sk, scale=D ** -0.5),
        in_specs=[pl.BlockSpec(memory_space=pl.ANY)] * 3,
        out_specs=pl.BlockSpec(memory_space=pl.ANY),
        out_shape=jax.ShapeDtypeStruct(oshape, q.dtype),
        scratch_shapes=[
            pltpu.VMEM((nh * Sq, D), q.dtype),
            pltpu.VMEM((_SLOTS, 2, Sk, D), k.dtype),
            pltpu.VMEM(oshape, q.dtype),
            pltpu.SemaphoreType.DMA((_SLOTS,)),
            pltpu.SemaphoreType.DMA((1,)),
        ],
        compiler_params=_params(),
    )(q.reshape(nh * Sq, D), k.reshape(nh, Sk, D), v.reshape(nh, Sk, D))
    return out.reshape(B, H, Sq, D)
```
